```python
import os as _os
_os.environ.setdefault("JAX_PLATFORMS", "cpu")
import jax
import jax.numpy as jnp

def _softmax(x, axis=-1):
    return jax.nn.softmax(x, axis=axis)
def _gelu(x):
    return jax.nn.gelu(x, approximate=True)
def _silu(x):
    return jax.nn.silu(x)
def _sigmoid(x):
    return jax.nn.sigmoid(x)
def _layernorm(x, axis=-1, eps=1e-5):
    m = jnp.mean(x, axis=axis, keepdims=True)
    v = jnp.var(x, axis=axis, keepdims=True)
    return (x - m) / jnp.sqrt(v + eps)
def _scatter_add(tgt, idx, src, axis=0):
    return tgt.at[idx].add(src)
def _segment_sum(src, seg, n):
    return jax.ops.segment_sum(src, seg, n)
class _Rng:
    def __init__(self, key):
        self._k = key
    def _next(self):
        self._k, sub = jax.random.split(self._k)
        return sub
    def normal(self, shape):
        return jax.random.normal(self._next(), shape, dtype=jnp.bfloat16)
    def randint(self, lo, hi, shape):
        return jax.random.randint(self._next(), shape, lo, hi, dtype=jnp.int32)
    def uniform(self, shape, lo=0.0, hi=1.0):
        return jax.random.uniform(self._next(), shape, jnp.bfloat16, lo, hi)
    def permutation(self, n):
        return jax.random.permutation(self._next(), n)


kernel_name = 'concat_heads__mha_block_cached__mha_block_cached__near_ridge'

def setup_inputs():
    _rng = _Rng(jax.random.key(int.from_bytes(__import__("os").urandom(4), "little")))
    _w = (lambda a: (lambda t: t.astype(jnp.bfloat16) if jnp.issubdtype(t.dtype, jnp.floating) else t)(jnp.asarray(a)))
    def _A_setup():
        B, Sq, D = 8, 144, 640
        H, Sk, Dh = 32, 512, 128
        return {
            "x": _w((lambda *s: _rng.normal(s) * 0.8)(B, Sq, D)),
            "k_cache": _w((lambda *s: _rng.normal(s) * 0.8)(B, H, Sk, Dh)),
            "v_cache": _w((lambda *s: _rng.normal(s) * 0.05)(B, H, Sk, Dh)),
            "wq": _w((lambda *s: _rng.normal(s) * 0.8)(D, H * Dh) * (D ** -0.5)),
            "wo": _w((lambda *s: _rng.normal(s) * 0.05)(H * Dh, D) * ((H * Dh) ** -0.5)),
        }
    _A_in = _A_setup()

    def _B_setup():
        B, Sq, D = 8, 144, 640
        H, Sk, Dh = 32, 512, 128
        return {
            "x": _w((lambda *s: _rng.normal(s) * 0.8)(B, Sq, D)),
            "k_cache": _w((lambda *s: _rng.normal(s) * 0.8)(B, H, Sk, Dh)),
            "v_cache": _w((lambda *s: _rng.normal(s) * 0.05)(B, H, Sk, Dh)),
            "wq": _w((lambda *s: _rng.normal(s) * 0.8)(D, H * Dh) * (D ** -0.5)),
            "wo": _w((lambda *s: _rng.normal(s) * 0.05)(H * Dh, D) * ((H * Dh) ** -0.5)),
        }
    _B_in = _B_setup()

    return {
        "A_x": _A_in["x"],
        "A_k_cache": _A_in["k_cache"],
        "A_v_cache": _A_in["v_cache"],
        "A_wq": _A_in["wq"],
        "A_wo": _A_in["wo"],
        "B_x": _B_in["x"],
        "B_k_cache": _B_in["k_cache"],
        "B_v_cache": _B_in["v_cache"],
        "B_wq": _B_in["wq"],
        "B_wo": _B_in["wo"],
    }

def reference(A_x, A_k_cache, A_v_cache, A_wq, A_wo, B_x, B_k_cache, B_v_cache, B_wq, B_wo):
    def _A_ref(x, k_cache, v_cache, wq, wo):
        B, Sq, D = x.shape
        H, Dh = 32, 128
        q = (lambda x, *d: x.transpose(*d))((x @ wq).reshape(B, Sq, H, Dh), 0, 2, 1, 3)
        scores = jnp.einsum("bhqd,bhkd->bhqk", q, k_cache) * (Dh ** -0.5)
        p = _softmax(scores, axis=-1)
        o = jnp.einsum("bhqk,bhkd->bhqd", p, v_cache)
        return (lambda x, *d: x.transpose(*d))(o, 0, 2, 1, 3).reshape(B, Sq, H * Dh) @ wo

    def _B_ref(x, k_cache, v_cache, wq, wo):
        B, Sq, D = x.shape
        H, Dh = 32, 128
        q = (lambda x, *d: x.transpose(*d))((x @ wq).reshape(B, Sq, H, Dh), 0, 2, 1, 3)
        scores = jnp.einsum("bhqd,bhkd->bhqk", q, k_cache) * (Dh ** -0.5)
        p = _softmax(scores, axis=-1)
        o = jnp.einsum("bhqk,bhkd->bhqd", p, v_cache)
        return (lambda x, *d: x.transpose(*d))(o, 0, 2, 1, 3).reshape(B, Sq, H * Dh) @ wo

    a = _A_ref(A_x, A_k_cache, A_v_cache, A_wq, A_wo)
    b = _B_ref(B_x, B_k_cache, B_v_cache, B_wq, B_wo)
    return jnp.concatenate([a, b], axis=-1)
```

```python
import jax
import jax.numpy as jnp
from jax import lax
import jax.experimental.pallas as pl
import jax.experimental.pallas.tpu as pltpu

_LOG2E = 1.4426950408889634
_NT = (((1,), (1,)), ((), ()))
_HG = 4
_NB = 4


@jax.jit
def pallas_concat_heads__mha_block_cached__mha_block_cached__near_ridge_kernel(
    A_x: jax.Array,
    A_k_cache: jax.Array,
    A_v_cache: jax.Array,
    A_wq: jax.Array,
    A_wo: jax.Array,
    B_x: jax.Array,
    B_k_cache: jax.Array,
    B_v_cache: jax.Array,
    B_wq: jax.Array,
    B_wo: jax.Array,
):
    B, Sq, D = A_x.shape
    _, H, Sk, Dh = A_k_cache.shape
    assert B == 8 and H % _HG == 0
    hg, nb = _HG, _NB
    G = H // hg
    NS = G * B
    L = nb - 1
    scale = (Dh ** -0.5) * _LOG2E
    BF, F32 = jnp.bfloat16, jnp.float32

    def kernel(xa, ka, va, wqa, woa, xb, kb, vb, wqb, wob, o_hbm,
               xbuf, kvbuf, wqbuf, wobuf, acc, obuf, xsem, kvsem, wqsem, wosem, osem):
        X = [xa, xb]
        KV = [ka, kb, va, vb]
        WQ = [wqa, wqb]
        WO = [woa, wob]

        def gb(s):
            if isinstance(s, int):
                return s >> 3, s & 7
            return lax.shift_right_logical(s, 3), s & 7

        def x_start(b, prio):
            for br in (0, 1):
                pltpu.make_async_copy(X[br].at[b], xbuf.at[b, br], xsem.at[b]).start(priority=prio)

        def x_wait(b):
            pltpu.make_async_copy(xbuf.at[b], xbuf.at[b], xsem.at[b]).wait()

        def kv_start(s, slot, prio):
            g, b = gb(s)
            for i in range(4):
                pltpu.make_async_copy(
                    KV[i].at[b, pl.ds(g * hg, hg)], kvbuf.at[slot, i], kvsem.at[slot]).start(priority=prio)

        def kv_wait(slot):
            pltpu.make_async_copy(kvbuf.at[slot], kvbuf.at[slot], kvsem.at[slot]).wait()

        def wq_start(g, prio):
            ws = g & 1
            for br in (0, 1):
                pltpu.make_async_copy(
                    WQ[br].at[:, pl.ds(pl.multiple_of(g * (hg * Dh), 128), hg * Dh)],
                    wqbuf.at[ws, br], wqsem.at[ws]).start(priority=prio)

        def wq_wait(ws):
            pltpu.make_async_copy(wqbuf.at[ws], wqbuf.at[ws], wqsem.at[ws]).wait()

        def wo_start(g, prio):
            ws = g & 1
            for br in (0, 1):
                pltpu.make_async_copy(
                    WO[br].at[pl.ds(pl.multiple_of(g * (hg * Dh), 128), hg * Dh), :],
                    wobuf.at[ws, br], wosem.at[ws]).start(priority=prio)

        def wo_wait(ws):
            pltpu.make_async_copy(wobuf.at[ws], wobuf.at[ws], wosem.at[ws]).wait()

        def o_copy(b):
            return pltpu.make_async_copy(obuf.at[b], o_hbm.at[b], osem.at[b])

        x_start(0, 0)
        wq_start(0, 0)
        kv_start(0, 0, 0)
        wo_start(0, 0)
        for j in range(1, L):
            x_start(j, 1)
            kv_start(j, j % nb, 1)
        acc[...] = jnp.zeros(acc.shape, F32)

        def step(s, carry):
            slot, nslot = carry
            g, b = gb(s)
            ws = g & 1

            @pl.when(g == 0)
            def _():
                x_wait(b)

            @pl.when(b == 0)
            def _():
                wq_wait(ws)
                wo_wait(ws)

            kv_wait(slot)

            def issue():
                sn = s + L

                @pl.when(sn < B)
                def _():
                    x_start(sn, 1)

                @pl.when(sn < NS)
                def _():
                    kv_start(sn, nslot, 1)

                @pl.when(jnp.logical_and(b == B - L, g + 1 < G))
                def _():
                    wq_start(g + 1, 1)
                    wo_start(g + 1, 1)

            q, p, l, o = {}, {}, {}, {}

            def qproj(br):
                r = jnp.dot(xbuf[b, br], wqbuf[ws, br], preferred_element_type=F32)
                q[br] = (r * scale).astype(BF)

            def qk(br, h):
                sc = lax.dot_general(q[br][:, h * Dh:(h + 1) * Dh], kvbuf[slot, br, h], _NT,
                                     preferred_element_type=F32)
                m = jnp.max(sc, axis=-1, keepdims=True)
                e = jnp.exp2(sc - m)
                l[br, h] = jnp.sum(e, axis=-1, keepdims=True)
                p[br, h] = e.astype(BF)

            def pv(br, h):
                r = pltpu.reciprocal(l[br, h], approx=True)
                r = r * (2.0 - l[br, h] * r)
                t = jnp.dot(p[br, h], kvbuf[slot, 2 + br, h], preferred_element_type=F32)
                o[br, h] = (t * r).astype(BF)

            def oproj(br):
                oo = jnp.concatenate([o[br, h] for h in range(hg)], axis=1)
                r = jnp.dot(oo, wobuf[ws, br], preferred_element_type=F32)
                acc[b, :, br * D:(br + 1) * D] += r

            jobs = [(br, h) for h in range(hg) for br in (0, 1)]
            qproj(0)
            issue()
            qproj(1)
            qk(*jobs[0])
            for i in range(len(jobs)):
                if i + 1 < len(jobs):
                    qk(*jobs[i + 1])
                pv(*jobs[i])
            oproj(0)
            oproj(1)

            @pl.when(g == G - 1)
            def _():
                obuf[b] = acc[b].astype(BF)
                o_copy(b).start()

            s1 = slot + 1
            n1 = nslot + 1
            return jnp.where(s1 == nb, 0, s1), jnp.where(n1 == nb, 0, n1)

        lax.fori_loop(0, NS, step, (jnp.int32(0), jnp.int32(L % nb)))
        for b in range(B):
            o_copy(b).wait()

    any_ = pl.BlockSpec(memory_space=pl.ANY)
    DMA = pltpu.SemaphoreType.DMA
    return pl.pallas_call(
        kernel,
        in_specs=[any_] * 10,
        out_specs=any_,
        out_shape=jax.ShapeDtypeStruct((B, Sq, 2 * D), BF),
        scratch_shapes=[
            pltpu.VMEM((B, 2, Sq, D), BF),
            pltpu.VMEM((nb, 4, hg, Sk, Dh), BF),
            pltpu.VMEM((2, 2, D, hg * Dh), BF),
            pltpu.VMEM((2, 2, hg * Dh, D), BF),
            pltpu.VMEM((B, Sq, 2 * D), F32),
            pltpu.VMEM((B, Sq, 2 * D), BF),
            DMA((B,)), DMA((nb,)), DMA((2,)), DMA((2,)), DMA((B,)),
        ],
        compiler_params=pltpu.CompilerParams(
            vmem_limit_bytes=100 * 2 ** 20, disable_bounds_checks=True),
    )(A_x, A_k_cache, A_v_cache, A_wq, A_wo, B_x, B_k_cache, B_v_cache, B_wq, B_wo)
```

```python
import jax
import jax.numpy as jnp
from jax import lax
import jax.experimental.pallas as pl
import jax.experimental.pallas.tpu as pltpu


_LOG2E = 1.4426950408889634
_NT = (((1,), (1,)), ((), ()))
_HG = 4
_LQP = 2
_NU = 12
_NQ = 32
_NW = 4


@jax.jit
def pallas_concat_heads__mha_block_cached__mha_block_cached__near_ridge_kernel(
    A_x: jax.Array,
    A_k_cache: jax.Array,
    A_v_cache: jax.Array,
    A_wq: jax.Array,
    A_wo: jax.Array,
    B_x: jax.Array,
    B_k_cache: jax.Array,
    B_v_cache: jax.Array,
    B_wq: jax.Array,
    B_wo: jax.Array,
):
    B, Sq, D = A_x.shape
    _, H, Sk, Dh = A_k_cache.shape
    assert (B, H) == (8, 32)
    hg, NU, NQ, NW, LQP = _HG, _NU, _NQ, _NW, _LQP
    G = H // hg
    NUNIT = G * B
    LQ = LQP * B
    NMAIN = NUNIT - LQ
    scale = (Dh ** -0.5) * _LOG2E
    BF, F32 = jnp.bfloat16, jnp.float32

    segs = ((2, 6, "q"), (4, 9, "q"), (4, 4, "tail"))
    groups = [
        [(0, 0, 0)],
        [(0, 0, 1)],
        [(0, 0, 2), (0, 0, 3)],
        [(0, 0, b) for b in range(4, 8)],
        [(1, 0, b) for b in range(0, 4)],
        [(1, 0, b) for b in range(4, 8)],
    ]
    ploop = 4

    def unit_gb(j):
        if j < NMAIN:
            return j >> 3, j & 7
        r = j - NMAIN
        return (G - LQP) + (r & 1), r >> 1

    steps = []
    u = 0
    for n, ns, _ in segs:
        for _t in range(ns):
            steps.append((u, n))
            u += n
    assert u == NUNIT
    tgt = []
    prev = NU - 1
    for u, n in steps:
        prev = max(prev, min(prev + n + 1, u - 1 + NU, NUNIT - 1))
        tgt.append(prev)

    def kernel(xa, ka, va, wqa, woa, xb, kb, vb, wqb, wob, o_hbm,
               xbuf, kvbuf, wqbuf, wobuf, qbufa, qbufb, acc, obuf, sems):
        X = [xa, xb]
        KV = [ka, kb, va, vb]
        WQ = [wqa, wqb]
        WO = [woa, wob]
        QB = [qbufa, qbufb]
        XS, KS = 0, 2 * B
        WQS = KS + NU
        WOS = WQS + 2 * NW
        OS = WOS + NW

        def x_copy(br, b):
            return pltpu.make_async_copy(X[br].at[b], xbuf.at[br, b], sems.at[XS + br * B + b])

        def kv_start(g, b, slot):
            for i in range(4):
                pltpu.make_async_copy(
                    KV[i].at[b, pl.ds(g * hg, hg)], kvbuf.at[slot, i], sems.at[KS + slot]).start()

        def kv_wait(slot):
            pltpu.make_async_copy(kvbuf.at[slot], kvbuf.at[slot], sems.at[KS + slot]).wait()

        def col0(g):
            c = g * (hg * Dh)
            return c if isinstance(g, int) else pl.multiple_of(c, hg * Dh)

        def wq_copy(br, g):
            ws = g & (NW - 1)
            return pltpu.make_async_copy(
                WQ[br].at[:, pl.ds(col0(g), hg * Dh)], wqbuf.at[ws, br], sems.at[WQS + 2 * ws + br])

        def wo_start(g):
            ws = g & (NW - 1)
            for br in (0, 1):
                pltpu.make_async_copy(
                    WO[br].at[pl.ds(col0(g), hg * Dh), :], wobuf.at[ws, br], sems.at[WOS + ws]).start()

        def wo_wait(g):
            ws = g & (NW - 1)
            pltpu.make_async_copy(wobuf.at[ws], wobuf.at[ws], sems.at[WOS + ws]).wait()

        def o_copy(b):
            return pltpu.make_async_copy(obuf.at[b], o_hbm.at[b], sems.at[OS + b])

        def when(c, f):
            if isinstance(c, bool):
                if c:
                    f()
            else:
                pl.when(c)(f)

        def land(a, b_):
            if isinstance(a, bool):
                return b_ if a else False
            return jnp.logical_and(a, b_)

        def wrap(v):
            return jnp.where(v >= NU, v - NU, v)

        def qproj(br, g, b, qslot):
            r = jnp.dot(xbuf[br, b], wqbuf[g & (NW - 1), br], preferred_element_type=F32)
            QB[br][qslot] = (r * scale).astype(BF)

        def attention(slot, qslot, hook=None):
            p, l, o = {}, {}, {}
            jobs = [(br, h) for h in range(hg) for br in (0, 1)]

            def qk(br, h):
                sc = lax.dot_general(QB[br][qslot, :, h * Dh:(h + 1) * Dh], kvbuf[slot, br, h], _NT,
                                     preferred_element_type=F32)
                m = jnp.max(sc, axis=-1, keepdims=True)
                e = jnp.exp2(sc - m)
                l[br, h] = jnp.sum(e, axis=-1, keepdims=True)
                p[br, h] = e.astype(BF)

            def pv(br, h):
                r = pltpu.reciprocal(l[br, h], approx=True)
                r = r * (2.0 - l[br, h] * r)
                t_ = jnp.dot(p[br, h], kvbuf[slot, 2 + br, h], preferred_element_type=F32)
                o[br, h] = (t_ * r).astype(BF)

            qk(*jobs[0])
            for i in range(len(jobs)):
                if i + 1 < len(jobs):
                    qk(*jobs[i + 1])
                if hook is not None and i == 1:
                    hook()
                pv(*jobs[i])
            return [jnp.concatenate([o[br, h] for h in range(hg)], axis=1) for br in (0, 1)]

        started = set()
        for grp in groups:
            for br, g, b in grp:
                if ("wq", br, g) not in started:
                    started.add(("wq", br, g))
                    wq_copy(br, g).start()
                x_copy(br, b).start()
        for br in (0, 1):
            wq_copy(br, 1).start()
        for j in range(NU):
            g, b = unit_gb(j)
            if b == 0:
                for br in (0, 1):
                    wq_copy(br, g + LQP).start()
                wo_start(g)
            kv_start(g, b, j)
        acc[...] = jnp.zeros(acc.shape, F32)
        waited = set()
        for grp in groups:
            for br, g, b in grp:
                if ("wq", br, g) not in waited:
                    waited.add(("wq", br, g))
                    wq_copy(br, g).wait()
                x_copy(br, b).wait()
            for br, g, b in grp:
                qproj(br, g, b, g * B + b)
        for br in (0, 1):
            wq_copy(br, 1).wait()

        def pstep(t, _):
            for i in range(ploop):
                b = t * ploop + i
                for br in (0, 1):
                    qproj(br, 1, b, B + b)

        lax.fori_loop(0, B // ploop, pstep, None)

        def segment(n, ns, kind, u0, t0):
            tgs = tgt[t0:t0 + ns]
            prevs = ([tgt[t0 - 1] if t0 > 0 else NU - 1] + tgs)[:ns]
            cnts = [a - b for a, b in zip(tgs, prevs)]
            mx = max(cnts)
            masks = [sum(1 << t for t in range(ns) if cnts[t] > i) for i in range(mx)]
            full = (1 << ns) - 1
            issued = [j for t in range(ns) for j in range(prevs[t] + 1, tgs[t] + 1)]
            main_w = any(j < NMAIN and j % B == 0 for j in issued)
            any_tail = any(j >= NMAIN for j in issued)
            tail_w = any(NMAIN <= j < NMAIN + LQP for j in issued)

            def step(t, carry):
                slot, nxt, nslot = carry
                u = u0 + t * n
                res = {"n": (nxt, nslot)}

                def issue():
                    j, sl = nxt, nslot
                    for i in range(mx):
                        if masks[i] == full:
                            act = True
                        else:
                            act = (lax.shift_right_logical(jnp.int32(masks[i]), t) & 1) == 1
                        ji, sli = j, sl
                        gi, bi = lax.shift_right_logical(ji, 3), ji & 7
                        if any_tail:
                            ist = ji >= NMAIN
                            r = ji - NMAIN
                            gi = jnp.where(ist, (G - LQP) + (r & 1), gi)
                            bi = jnp.where(ist, lax.shift_right_arithmetic(r, 1), bi)
                        if main_w:
                            def fw():
                                for br in (0, 1):
                                    wq_copy(br, gi + LQP).start()
                                wo_start(gi)
                            c = jnp.logical_and(bi == 0, ji < NMAIN) if any_tail else bi == 0
                            when(land(act, c), fw)
                        if tail_w:
                            when(land(act, jnp.logical_and(bi == 0, ist)), lambda: wo_start(gi))
                        when(act, lambda: kv_start(gi, bi, sli))
                        inc = 1 if act is True else act.astype(jnp.int32)
                        j = j + inc
                        sl = wrap(sl + inc)
                    res["n"] = (j, sl)

                if kind == "q":
                    g = lax.shift_right_logical(u, 3)
                    b0 = u & 7

                    def fw():
                        for br in (0, 1):
                            wq_copy(br, g + LQP).wait()
                        wo_wait(g)

                    when(b0 == 0, fw)
                    for i in range(n):
                        kv_wait(slot + i)
                    ws = g & (NW - 1)
                    for i in range(n):
                        b = b0 + i
                        qs = (u + i + LQ) & (NQ - 1)
                        qproj(1, g + LQP, b, qs)
                        if i == 0:
                            issue()
                        oc = attention(slot + i, (u + i) & (NQ - 1))
                        for br in (0, 1):
                            r = jnp.dot(oc[br], wobuf[ws, br], preferred_element_type=F32)
                            acc[b, :, br * D:(br + 1) * D] += r
                            if br == 0:
                                qproj(0, g + LQP, b, qs)
                else:
                    b0 = t * (n // 2)

                    def fw():
                        wo_wait(G - 2)
                        wo_wait(G - 1)

                    when(t == 0, fw)
                    for i in range(n):
                        kv_wait(slot + i)
                    for i in range(n):
                        b = b0 + i // 2
                        g = G - 2 + (i & 1)
                        oc = attention(slot + i, (g * B + b) & (NQ - 1),
                                       issue if (i == 0 and mx > 0) else None)
                        for br in (0, 1):
                            r = jnp.dot(oc[br], wobuf[g & (NW - 1), br], preferred_element_type=F32)
                            cs = slice(br * D, (br + 1) * D)
                            if i & 1 == 0:
                                acc[b, :, cs] += r
                            else:
                                obuf[b, :, cs] = (acc[b, :, cs] + r).astype(BF)
                        if i & 1:
                            o_copy(b).start()
                return (wrap(slot + n),) + res["n"]

            return step

        u0 = 0
        t0 = 0
        for n, ns, kind in segs:
            nxt = (tgt[t0 - 1] if t0 > 0 else NU - 1) + 1
            carry = (jnp.int32(u0 % NU), jnp.int32(nxt), jnp.int32(nxt % NU))
            lax.fori_loop(0, ns, segment(n, ns, kind, u0, t0), carry)
            u0 += n * ns
            t0 += ns
        for b in range(B):
            o_copy(b).wait()

    any_ = pl.BlockSpec(memory_space=pl.ANY)
    return pl.pallas_call(
        kernel,
        in_specs=[any_] * 10,
        out_specs=any_,
        out_shape=jax.ShapeDtypeStruct((B, Sq, 2 * D), BF),
        scratch_shapes=[
            pltpu.VMEM((2, B, Sq, D), BF),
            pltpu.VMEM((NU, 4, hg, Sk, Dh), BF),
            pltpu.VMEM((NW, 2, D, hg * Dh), BF),
            pltpu.VMEM((NW, 2, hg * Dh, D), BF),
            pltpu.VMEM((NQ, Sq, hg * Dh), BF),
            pltpu.VMEM((NQ, Sq, hg * Dh), BF),
            pltpu.VMEM((B, Sq, 2 * D), F32),
            pltpu.VMEM((B, Sq, 2 * D), BF),
            pltpu.SemaphoreType.DMA((2 * B + NU + 3 * NW + B,)),
        ],
        compiler_params=pltpu.CompilerParams(
            vmem_limit_bytes=100 * 2 ** 20, disable_bounds_checks=True),
    )(A_x, A_k_cache, A_v_cache, A_wq, A_wo, B_x, B_k_cache, B_v_cache, B_wq, B_wo)
```

```python
import jax
import jax.numpy as jnp
from jax import lax
import jax.experimental.pallas as pl
import jax.experimental.pallas.tpu as pltpu


_LOG2E = 1.4426950408889634
_NT = (((1,), (1,)), ((), ()))
_HG = 4
_NU = 8
_NQ = 32
_NW = 4
_LQP = 2


@jax.jit
def pallas_concat_heads__mha_block_cached__mha_block_cached__near_ridge_kernel(
    A_x: jax.Array,
    A_k_cache: jax.Array,
    A_v_cache: jax.Array,
    A_wq: jax.Array,
    A_wo: jax.Array,
    B_x: jax.Array,
    B_k_cache: jax.Array,
    B_v_cache: jax.Array,
    B_wq: jax.Array,
    B_wo: jax.Array,
):
    B, Sq, D = A_x.shape
    _, H, Sk, Dh = A_k_cache.shape
    hg, NU, NQ, NW, LQP = _HG, _NU, _NQ, _NW, _LQP
    G = H // hg
    assert B == NU == 8 and G == 8 and D % 128 == 0
    NUNIT = G * B
    LQ = LQP * B
    NMAIN = NUNIT - LQ
    LA = NU - 1
    NT_UNITS = 4
    scale = (Dh ** -0.5) * _LOG2E
    BF, F32 = jnp.bfloat16, jnp.float32
    pieces = [(0, D)] + [(D + c, D + c + 128) for c in range(0, D, 128)]

    def unit_gb(j):
        if j < NMAIN:
            return j // B, j % B
        r = j - NMAIN
        return (G - LQP) + (r & 1), r >> 1

    def kernel(xa, ka, va, wqa, woa, xb, kb, vb, wqb, wob, o_hbm,
               xbuf, kvbuf, wqbuf, wobuf, qbufa, qbufb, acc, obuf, sems):
        X = [xa, xb]
        KV = [ka, kb, va, vb]
        WQ = [wqa, wqb]
        WO = [woa, wob]
        QB = [qbufa, qbufb]
        XS, KS = 0, 2 * B
        WQS = KS + NU
        WOS = WQS + 2 * NW
        OS = WOS + NW

        def x_copy(br, b):
            return pltpu.make_async_copy(X[br].at[b], xbuf.at[br, b], sems.at[XS + br * B + b])

        def kv_start(g, b, slot):
            for i in range(4):
                pltpu.make_async_copy(
                    KV[i].at[b, pl.ds(g * hg, hg)], kvbuf.at[slot, i], sems.at[KS + slot]).start()

        def kv_wait(slot):
            pltpu.make_async_copy(kvbuf.at[slot], kvbuf.at[slot], sems.at[KS + slot]).wait()

        def col0(g):
            c = g * (hg * Dh)
            return c if isinstance(g, int) else pl.multiple_of(c, hg * Dh)

        def wq_copy(br, g):
            ws = g & (NW - 1)
            return pltpu.make_async_copy(
                WQ[br].at[:, pl.ds(col0(g), hg * Dh)], wqbuf.at[ws, br], sems.at[WQS + 2 * ws + br])

        def wo_start(g):
            ws = g & (NW - 1)
            for br in (0, 1):
                pltpu.make_async_copy(
                    WO[br].at[pl.ds(col0(g), hg * Dh), :], wobuf.at[ws, br], sems.at[WOS + ws]).start()

        def wo_wait(g):
            ws = g & (NW - 1)
            pltpu.make_async_copy(wobuf.at[ws], wobuf.at[ws], sems.at[WOS + ws]).wait()

        def o_copy(b, pi):
            lo, hi = pieces[pi]
            return pltpu.make_async_copy(
                obuf.at[b, :, lo:hi], o_hbm.at[b, :, lo:hi], sems.at[OS + b * len(pieces) + pi])

        def qproj(br, g, b, qslot):
            r = jnp.dot(xbuf[br, b], wqbuf[g & (NW - 1), br], preferred_element_type=F32)
            QB[br][qslot] = (r * scale).astype(BF)

        def attention(slot, qslot, hook=None):
            p, l, o = {}, {}, {}
            jobs = [(br, h) for h in range(hg) for br in (0, 1)]

            def qk(br, h):
                sc = lax.dot_general(QB[br][qslot, :, h * Dh:(h + 1) * Dh], kvbuf[slot, br, h], _NT,
                                     preferred_element_type=F32)
                m = jnp.max(sc, axis=-1, keepdims=True)
                e = jnp.exp2(sc - m)
                l[br, h] = jnp.sum(e, axis=-1, keepdims=True)
                p[br, h] = e.astype(BF)

            def pv(br, h):
                r = pltpu.reciprocal(l[br, h], approx=True)
                r = r * (2.0 - l[br, h] * r)
                t_ = jnp.dot(p[br, h], kvbuf[slot, 2 + br, h], preferred_element_type=F32)
                o[br, h] = (t_ * r).astype(BF)

            qk(*jobs[0])
            for i in range(len(jobs)):
                if i + 1 < len(jobs):
                    qk(*jobs[i + 1])
                if hook is not None and i == 1:
                    hook()
                pv(*jobs[i])
            return [jnp.concatenate([o[br, h] for h in range(hg)], axis=1) for br in (0, 1)]

        for g in range(LQP):
            for br in (0, 1):
                wq_copy(br, g).start()
                if g == 0:
                    for b in range(B):
                        x_copy(br, b).start()
        for j in range(LA):
            g, b = unit_gb(j)
            kv_start(g, b, j)
            if b == 0:
                for br in (1, 0):
                    wq_copy(br, g + LQP).start()
                wo_start(g)

        def zstep(b, _):
            acc[b] = jnp.zeros((Sq, 2 * D), F32)

        lax.fori_loop(0, B, zstep, None)

        def pstep(g, _):
            for br in (0, 1):
                wq_copy(br, g).wait()
                for b in range(B):
                    pl.when(g == 0)(lambda: x_copy(br, b).wait())
                    qproj(br, g, b, g * B + b)

        lax.fori_loop(0, LQP, pstep, None)

        def mstep(g, _):
            ws = g & (NW - 1)
            last = g == G - LQP - 1
            for b in range(B):
                qs = (g * B + b + LQ) & (NQ - 1)
                if b == 0:
                    wq_copy(1, g + LQP).wait()
                qproj(1, g + LQP, b, qs)
                if b == 0:
                    kv_start(g, B - 1, B - 1)
                else:
                    r = b - 1
                    gi = g + 1 if r & 1 == 0 else jnp.where(last, G - 1, g + 1)
                    bi = r if r == 0 else jnp.where(last, r >> 1, r)
                    kv_start(gi, bi, r)
                    if b == 1:
                        @pl.when(jnp.logical_not(last))
                        def _():
                            for br in (1, 0):
                                wq_copy(br, g + 1 + LQP).start()
                        wo_start(g + 1)
                    if b == 2:
                        pl.when(last)(lambda: wo_start(G - 1))
                kv_wait(b)
                oc = attention(b, (g * B + b) & (NQ - 1))
                if b == 0:
                    wo_wait(g)
                for br in (0, 1):
                    rr = jnp.dot(oc[br], wobuf[ws, br], preferred_element_type=F32)
                    acc[b, :, br * D:(br + 1) * D] += rr
                    if br == 0:
                        if b == 0:
                            wq_copy(0, g + LQP).wait()
                        qproj(0, g + LQP, b, qs)

        lax.fori_loop(0, G - LQP, mstep, None)

        nst = LQ // NT_UNITS

        def tstep(t, _):
            for i in range(NT_UNITS):
                u = NMAIN + t * NT_UNITS + i
                b = t * (NT_UNITS // 2) + i // 2
                g = G - 2 + (i & 1)

                def issue():
                    j = u + LA
                    r = j - NMAIN
                    go = lambda: kv_start((G - LQP) + (r & 1), lax.shift_right_arithmetic(r, 1), j & (NU - 1))
                    pl.when(j < NUNIT)(go)

                if i == 0:
                    kv_wait(u & (NU - 1))
                oc = attention(u & (NU - 1), (g * B + b) & (NQ - 1), issue)
                if i + 1 < NT_UNITS:
                    kv_wait((u + 1) & (NU - 1))
                if i < 2:
                    pl.when(t == 0)(lambda: wo_wait(g))
                if i & 1 == 0:
                    for br in (0, 1):
                        rr = jnp.dot(oc[br], wobuf[g & (NW - 1), br], preferred_element_type=F32)
                        acc[b, :, br * D:(br + 1) * D] += rr
                else:
                    rr = jnp.dot(oc[0], wobuf[g & (NW - 1), 0], preferred_element_type=F32)
                    obuf[b, :, 0:D] = (acc[b, :, 0:D] + rr).astype(BF)
                    o_copy(b, 0).start()
                    for pi, (lo, hi) in enumerate(pieces[1:], start=1):
                        rr = jnp.dot(oc[1], wobuf[g & (NW - 1), 1, :, lo - D:hi - D],
                                     preferred_element_type=F32)
                        obuf[b, :, lo:hi] = (acc[b, :, lo:hi] + rr).astype(BF)
                        o_copy(b, pi).start()

        lax.fori_loop(0, nst, tstep, None)
        for b in range(B):
            for pi in range(len(pieces)):
                o_copy(b, pi).wait()

    any_ = pl.BlockSpec(memory_space=pl.ANY)
    return pl.pallas_call(
        kernel,
        in_specs=[any_] * 10,
        out_specs=any_,
        out_shape=jax.ShapeDtypeStruct((B, Sq, 2 * D), BF),
        scratch_shapes=[
            pltpu.VMEM((2, B, Sq, D), BF),
            pltpu.VMEM((NU, 4, hg, Sk, Dh), BF),
            pltpu.VMEM((NW, 2, D, hg * Dh), BF),
            pltpu.VMEM((NW, 2, hg * Dh, D), BF),
            pltpu.VMEM((NQ, Sq, hg * Dh), BF),
            pltpu.VMEM((NQ, Sq, hg * Dh), BF),
            pltpu.VMEM((B, Sq, 2 * D), F32),
            pltpu.VMEM((B, Sq, 2 * D), BF),
            pltpu.SemaphoreType.DMA((2 * B + NU + 3 * NW + B * len(pieces),)),
        ],
        compiler_params=pltpu.CompilerParams(
            vmem_limit_bytes=100 * 2 ** 20,
            flags={"XLA_TPU_RESCHEDULE_DMA_DONES": True},
            disable_bounds_checks=True,
            disable_semaphore_checks=True,
        ),
    )(A_x, A_k_cache, A_v_cache, A_wq, A_wo, B_x, B_k_cache, B_v_cache, B_wq, B_wo)
```

```python
import jax
import jax.numpy as jnp
from jax import lax
import jax.experimental.pallas as pl
import jax.experimental.pallas.tpu as pltpu


_LOG2E = 1.4426950408889634
_NT = (((1,), (1,)), ((), ()))
_HG = 4
_NU = 8
_NQ = 32
_NW = 4
_LQP = 2


@jax.jit
def pallas_concat_heads__mha_block_cached__mha_block_cached__near_ridge_kernel(
    A_x: jax.Array,
    A_k_cache: jax.Array,
    A_v_cache: jax.Array,
    A_wq: jax.Array,
    A_wo: jax.Array,
    B_x: jax.Array,
    B_k_cache: jax.Array,
    B_v_cache: jax.Array,
    B_wq: jax.Array,
    B_wo: jax.Array,
):
    B, Sq, D = A_x.shape
    _, H, Sk, Dh = A_k_cache.shape
    hg, NU, NQ, NW, LQP = _HG, _NU, _NQ, _NW, _LQP
    G = H // hg
    assert B == NU == 8 and G == 8 and D % 128 == 0
    NUNIT = G * B
    LQ = LQP * B
    NMAIN = NUNIT - LQ
    LA = NU - 1
    NT_UNITS = 4
    NKC = D // 128
    scale = (Dh ** -0.5) * _LOG2E
    BF, F32 = jnp.bfloat16, jnp.float32
    pieces = [(0, D)] + [(D + c, D + c + 128) for c in range(0, D, 128)]

    def unit_gb(j):
        if j < NMAIN:
            return j // B, j % B
        r = j - NMAIN
        return (G - LQP) + (r & 1), r >> 1

    def kernel(xa, ka, va, wqa, woa, xb, kb, vb, wqb, wob, o_hbm,
               xbuf, kvbuf, wqbuf, wobuf, qbufa, qbufb, acc, obuf, sems):
        X = [xa, xb]
        KV = [ka, kb, va, vb]
        WQ = [wqa, wqb]
        WO = [woa, wob]
        QB = [qbufa, qbufb]
        XS, KS = 0, 2 * B
        WQS = KS + NU
        WOS = WQS + 2 * NW
        OS = WOS + NW
        CS = OS + B * len(pieces)

        def x_copy(br, b):
            return pltpu.make_async_copy(X[br].at[b], xbuf.at[br, b], sems.at[XS + br * B + b])

        def kv_start(g, b, slot):
            for i in range(4):
                pltpu.make_async_copy(
                    KV[i].at[b, pl.ds(g * hg, hg)], kvbuf.at[slot, i], sems.at[KS + slot]).start()

        def kv_wait(slot):
            pltpu.make_async_copy(kvbuf.at[slot], kvbuf.at[slot], sems.at[KS + slot]).wait()

        def col0(g):
            c = g * (hg * Dh)
            return c if isinstance(g, int) else pl.multiple_of(c, hg * Dh)

        def wq_copy(br, g):
            ws = g & (NW - 1)
            return pltpu.make_async_copy(
                WQ[br].at[:, pl.ds(col0(g), hg * Dh)], wqbuf.at[ws, br], sems.at[WQS + 2 * ws + br])

        def wq_chunk(g, c):
            return pltpu.make_async_copy(
                wqa.at[c * 128:(c + 1) * 128, pl.ds(col0(g), hg * Dh)],
                wqbuf.at[g & (NW - 1), 0, c * 128:(c + 1) * 128], sems.at[CS + g * NKC + c])

        def wo_start(g):
            ws = g & (NW - 1)
            for br in (0, 1):
                pltpu.make_async_copy(
                    WO[br].at[pl.ds(col0(g), hg * Dh), :], wobuf.at[ws, br], sems.at[WOS + ws]).start()

        def wo_wait(g):
            ws = g & (NW - 1)
            pltpu.make_async_copy(wobuf.at[ws], wobuf.at[ws], sems.at[WOS + ws]).wait()

        def o_copy(b, pi):
            lo, hi = pieces[pi]
            return pltpu.make_async_copy(
                obuf.at[b, :, lo:hi], o_hbm.at[b, :, lo:hi], sems.at[OS + b * len(pieces) + pi])

        def qproj(br, g, b, qslot):
            r = jnp.dot(xbuf[br, b], wqbuf[g & (NW - 1), br], preferred_element_type=F32)
            QB[br][qslot] = (r * scale).astype(BF)

        def attention(slot, qslot, hook, hpos):
            p, l, o = {}, {}, {}
            jobs = [(br, h) for br in (0, 1) for h in range(hg)]

            def qk(br, h):
                sc = lax.dot_general(QB[br][qslot, :, h * Dh:(h + 1) * Dh], kvbuf[slot, br, h], _NT,
                                     preferred_element_type=F32)
                m = jnp.max(sc, axis=-1, keepdims=True)
                e = jnp.exp2(sc - m)
                l[br, h] = jnp.sum(e, axis=-1, keepdims=True)
                p[br, h] = e.astype(BF)

            def pv(br, h):
                r = pltpu.reciprocal(l[br, h], approx=True)
                r = r * (2.0 - l[br, h] * r)
                t_ = jnp.dot(p[br, h], kvbuf[slot, 2 + br, h], preferred_element_type=F32)
                o[br, h] = (t_ * r).astype(BF)

            qk(*jobs[0])
            for i in range(len(jobs)):
                if i + 1 < len(jobs):
                    qk(*jobs[i + 1])
                if i == hpos:
                    hook()
                pv(*jobs[i])
            return [jnp.concatenate([o[br, h] for h in range(hg)], axis=1) for br in (0, 1)]

        x_copy(0, 0).start()
        for c in range(NKC):
            if c == 2:
                x_copy(0, 1).start()
            wq_chunk(0, c).start()
        for b in range(2, B):
            x_copy(0, b).start()
        wq_copy(1, 0).start()
        for b in range(B):
            x_copy(1, b).start()
        for c in range(NKC):
            wq_chunk(1, c).start()
        wq_copy(1, 1).start()
        for j in range(LA):
            g, b = unit_gb(j)
            kv_start(g, b, j)
            if b == 0:
                for br in (1, 0):
                    wq_copy(br, g + LQP).start()
                wo_start(g)

        def zstep(b, _):
            acc[b] = jnp.zeros((Sq, 2 * D), F32)

        lax.fori_loop(0, B, zstep, None)

        def pstep(g, _):
            first = g == 0
            part = {}

            def chunk(b, c):
                ks = slice(c * 128, (c + 1) * 128)
                d = jnp.dot(xbuf[0, b, :, ks], wqbuf[g & (NW - 1), 0, ks, :], preferred_element_type=F32)
                part[b] = part[b] + d if b in part else d

            pl.when(first)(lambda: x_copy(0, 0).wait())
            for c in range(NKC):
                if c == 2:
                    pl.when(first)(lambda: x_copy(0, 1).wait())
                    for cc in range(c):
                        chunk(1, cc)
                wq_chunk(g, c).wait()
                chunk(0, c)
                if c >= 2:
                    chunk(1, c)
            for b in range(2):
                qbufa[g * B + b] = (part[b] * scale).astype(BF)
            for br in (0, 1):
                if br == 1:
                    wq_copy(br, g).wait()
                for b in range(2 if br == 0 else 0, B):
                    pl.when(first)(lambda: x_copy(br, b).wait())
                    qproj(br, g, b, g * B + b)

        lax.fori_loop(0, LQP, pstep, None)

        def mstep(g, _):
            ws = g & (NW - 1)
            last = g == G - LQP - 1
            for b in range(B):
                qs = (g * B + b + LQ) & (NQ - 1)
                if b == 0:
                    wq_copy(1, g + LQP).wait()
                qproj(1, g + LQP, b, qs)

                def issue():
                    if b == 0:
                        kv_start(g, B - 1, B - 1)
                    else:
                        r = b - 1
                        gi = g + 1 if r & 1 == 0 else jnp.where(last, G - 1, g + 1)
                        bi = r if r == 0 else jnp.where(last, r >> 1, r)
                        kv_start(gi, bi, r)
                        if b == 1:
                            @pl.when(jnp.logical_not(last))
                            def _():
                                for br in (1, 0):
                                    wq_copy(br, g + 1 + LQP).start()
                            wo_start(g + 1)
                        if b == 2:
                            pl.when(last)(lambda: wo_start(G - 1))

                kv_wait(b)
                oc = attention(b, (g * B + b) & (NQ - 1), issue, 2)
                if b == 0:
                    wo_wait(g)
                for br in (0, 1):
                    rr = jnp.dot(oc[br], wobuf[ws, br], preferred_element_type=F32)
                    acc[b, :, br * D:(br + 1) * D] += rr
                    if br == 0:
                        if b == 0:
                            wq_copy(0, g + LQP).wait()
                        qproj(0, g + LQP, b, qs)

        lax.fori_loop(0, G - LQP, mstep, None)

        nst = LQ // NT_UNITS

        def tstep(t, _):
            for i in range(NT_UNITS):
                u = NMAIN + t * NT_UNITS + i
                b = t * (NT_UNITS // 2) + i // 2
                g = G - 2 + (i & 1)

                def issue():
                    j = u + LA

                    @pl.when(j < NUNIT)
                    def _():
                        r = j - NMAIN
                        kv_start((G - LQP) + (r & 1), lax.shift_right_arithmetic(r, 1), j & (NU - 1))

                if i == 0:
                    kv_wait(u & (NU - 1))
                oc = attention(u & (NU - 1), (g * B + b) & (NQ - 1), issue, 1)
                if i + 1 < NT_UNITS:
                    kv_wait((u + 1) & (NU - 1))
                if i < 2:
                    pl.when(t == 0)(lambda: wo_wait(g))
                if i & 1 == 0:
                    for br in (0, 1):
                        rr = jnp.dot(oc[br], wobuf[g & (NW - 1), br], preferred_element_type=F32)
                        acc[b, :, br * D:(br + 1) * D] += rr
                else:
                    rr = jnp.dot(oc[0], wobuf[g & (NW - 1), 0], preferred_element_type=F32)
                    obuf[b, :, 0:D] = (acc[b, :, 0:D] + rr).astype(BF)
                    o_copy(b, 0).start()
                    for pi, (lo, hi) in enumerate(pieces[1:], start=1):
                        rr = jnp.dot(oc[1], wobuf[g & (NW - 1), 1, :, lo - D:hi - D],
                                     preferred_element_type=F32)
                        obuf[b, :, lo:hi] = (acc[b, :, lo:hi] + rr).astype(BF)
                        o_copy(b, pi).start()

        lax.fori_loop(0, nst, tstep, None)
        for b in range(B):
            for pi in range(len(pieces)):
                o_copy(b, pi).wait()

    any_ = pl.BlockSpec(memory_space=pl.ANY)
    return pl.pallas_call(
        kernel,
        in_specs=[any_] * 10,
        out_specs=any_,
        out_shape=jax.ShapeDtypeStruct((B, Sq, 2 * D), BF),
        scratch_shapes=[
            pltpu.VMEM((2, B, Sq, D), BF),
            pltpu.VMEM((NU, 4, hg, Sk, Dh), BF),
            pltpu.VMEM((NW, 2, D, hg * Dh), BF),
            pltpu.VMEM((NW, 2, hg * Dh, D), BF),
            pltpu.VMEM((NQ, Sq, hg * Dh), BF),
            pltpu.VMEM((NQ, Sq, hg * Dh), BF),
            pltpu.VMEM((B, Sq, 2 * D), F32),
            pltpu.VMEM((B, Sq, 2 * D), BF),
            pltpu.SemaphoreType.DMA((2 * B + NU + 3 * NW + B * len(pieces) + LQP * NKC,)),
        ],
        compiler_params=pltpu.CompilerParams(
            vmem_limit_bytes=100 * 2 ** 20,
            flags={"XLA_TPU_RESCHEDULE_DMA_DONES": True},
            disable_bounds_checks=True,
            disable_semaphore_checks=True,
        ),
    )(A_x, A_k_cache, A_v_cache, A_wq, A_wo, B_x, B_k_cache, B_v_cache, B_wq, B_wo)
```
